```python
import os as _os
_os.environ.setdefault('JAX_PLATFORMS', 'cpu')
import jax
import jax.numpy as jnp

def _softmax(x, axis=-1):
    return jax.nn.softmax(x, axis=axis)

def _gelu(x):
    return jax.nn.gelu(x, approximate=True)

def _silu(x):
    return jax.nn.silu(x)

def _sigmoid(x):
    return jax.nn.sigmoid(x)

def _layernorm(x, axis=-1, eps=1e-05):
    m = jnp.mean(x, axis=axis, keepdims=True)
    v = jnp.var(x, axis=axis, keepdims=True)
    return (x - m) / jnp.sqrt(v + eps)

def _scatter_add(tgt, idx, src, axis=0):
    return tgt.at[idx].add(src)

def _segment_sum(src, seg, n):
    return jax.ops.segment_sum(src, seg, n)

class _Rng:

    def __init__(self, key):
        self._k = key

    def _next(self):
        self._k, sub = jax.random.split(self._k)
        return sub

    def normal(self, shape):
        return jax.random.normal(self._next(), shape, dtype=jnp.bfloat16)

    def randint(self, lo, hi, shape):
        return jax.random.randint(self._next(), shape, lo, hi, dtype=jnp.int32)

    def uniform(self, shape, lo=0.0, hi=1.0):
        return jax.random.uniform(self._next(), shape, jnp.bfloat16, lo, hi)

    def permutation(self, n):
        return jax.random.permutation(self._next(), n)
kernel_name = 'gated_mix__sliding_block__memory_aug_recurrent_mem_tr__prompt'

def setup_inputs():
    _rng = _Rng(jax.random.key(int.from_bytes(__import__("os").urandom(4), "little")))
    _w = lambda a: (lambda t: t.astype(jnp.bfloat16) if jnp.issubdtype(t.dtype, jnp.floating) else t)(jnp.asarray(a))

    def _A_setup():
        B, S, D = (1, 2048, 448)
        return {'x': _w((lambda *s: _rng.normal(s) * 0.05)(B, S, D)), 'wqkv': _w((lambda *s: _rng.normal(s) * 0.8)(D, 3 * D)), 'wo': _w((lambda *s: _rng.normal(s) * 0.05)(D, D))}
    _A_in = _A_setup()

    def _B_setup():
        B, S, Dm = (1, 2048, 448)
        H, Dh = (16, 256)
        M, seg = (8, 32)
        seg = min(seg, S)
        S = S // seg * seg
        return {'x': _w((lambda *s: _rng.normal(s) * 0.05)(B, S, Dm)), 'mem0': _w((lambda *s: _rng.normal(s) * 0.8)(B, M, Dm)), 'Wq': _w((lambda *s: _rng.normal(s) * 3.2)(Dm, H, Dh) * Dm ** (-0.5)), 'Wk': _w((lambda *s: _rng.normal(s) * 3.2)(Dm, H, Dh) * Dm ** (-0.5)), 'Wv': _w((lambda *s: _rng.normal(s) * 0.8)(Dm, H, Dh) * Dm ** (-0.5)), 'Wo': _w((lambda *s: _rng.normal(s) * 0.8)(H, Dh, Dm) * (H * Dh) ** (-0.5)), 'seg_len': seg}
    _B_in = _B_setup()
    return {'A_x': _A_in['x'], 'A_wqkv': _A_in['wqkv'], 'A_wo': _A_in['wo'], 'B_x': _B_in['x'], 'B_mem0': _B_in['mem0'], 'B_Wq': _B_in['Wq'], 'B_Wk': _B_in['Wk'], 'B_Wv': _B_in['Wv'], 'B_Wo': _B_in['Wo'], 'B_seg_len': _B_in['seg_len'], 'gate_w': _w((lambda *s: _rng.normal(s) * 0.05)(448) * 16.0)}

def reference(A_x, A_wqkv, A_wo, B_x, B_mem0, B_Wq, B_Wk, B_Wv, B_Wo, B_seg_len, gate_w):

    def _A_ref(x, wqkv, wo):
        B, S, D = x.shape
        H = 16
        Dh = D // H
        W = 256
        qkv = (lambda x, *d: x.transpose(*d))((x @ wqkv).reshape(B, S, 3, H, Dh), 2, 0, 3, 1, 4)
        q, k, v = (qkv[0], qkv[1], qkv[2])
        scores = jnp.einsum('bhqd,bhkd->bhqk', q, k) * Dh ** (-0.5)
        idx = jnp.arange(S)
        mask = (idx[:, None] - idx[None, :] >= 0) & (idx[:, None] - idx[None, :] < W)
        scores = jnp.where(mask[None, None], scores, -1000000000.0)
        p = _softmax(scores, axis=-1)
        o = jnp.einsum('bhqk,bhkd->bhqd', p, v)
        return (lambda x, *d: x.transpose(*d))(o, 0, 2, 1, 3).reshape(B, S, D) @ wo

    def _B_ref(x, mem0, Wq, Wk, Wv, Wo, seg_len):
        B, S, Dm = x.shape
        H, Dh = (Wq.shape[1], Wq.shape[2])
        M = mem0.shape[1]
        scale = Dh ** (-0.5)
        n_seg = S // seg_len
        L = M + seg_len
        idx = jnp.arange(L)
        mask = (idx[:, None] < M) | (idx[:, None] >= idx[None, :])
        mem = mem0
        outs = []
        for s in range(n_seg):
            xs = x[:, s * seg_len:(s + 1) * seg_len, :].copy()
            h = jnp.concatenate([mem, xs], axis=1)
            q = jnp.einsum('btd,dhe->bhte', h, Wq)
            k = jnp.einsum('btd,dhe->bhte', h, Wk)
            v = jnp.einsum('btd,dhe->bhte', h, Wv)
            scores = jnp.einsum('bhqe,bhke->bhqk', q, k) * scale
            scores = jnp.where(mask[None, None], scores, -1000000000.0)
            p = _softmax(scores, axis=-1)
            o = jnp.einsum('bhqk,bhke->bhqe', p, v)
            o = jnp.einsum('bhte,hed->btd', o, Wo)
            mem = o[:, :M, :].copy()
            outs.append(o[:, M:, :])
        return jnp.concatenate(outs, axis=1)
    x = A_x
    g = _sigmoid((x * gate_w).sum(-1, keepdims=True))
    a = _A_ref(x, A_wqkv, A_wo)
    b = _B_ref(x, B_mem0, B_Wq, B_Wk, B_Wv, B_Wo, B_seg_len)
    return g * a + (1 - g) * b
```

```python
import functools
import jax
import jax.numpy as jnp
from jax import lax
import jax.experimental.pallas as pl
import jax.experimental.pallas.tpu as pltpu

F32 = jnp.float32
BF16 = jnp.bfloat16
U32 = jnp.uint32

S = 2048
D = 448
HA = 16
DHA = 28
DP = 32
WIN = 256
HB = 16
DHB = 256
MEM = 8
SEG = 32
NSEG = S // SEG
NEG = -1e30
LOG2E = 1.4426950408889634
AFILL = 1
FILLH = 1
FILLH2 = 6
FILLH3 = 11


def _dot(a, b):
    return jnp.dot(a, b, preferred_element_type=F32)


def _dot_nt(a, b):
    return lax.dot_general(a, b, (((1,), (1,)), ((), ())), preferred_element_type=F32)


def _pk(x):
    return pltpu.bitcast(x, U32)


def _upk(x):
    return pltpu.bitcast(x, BF16)


def _recip(x):
    r = pl.reciprocal(x, approx=True)
    return r * (2.0 - x * r)


def _cat(parts):
    return jnp.concatenate(parts, axis=0)


def _kernel(xaT_hbm, wqkv_hbm, wo_hbm, gate_hbm, mem0_hbm, wq_hbm, wk_hbm, wv_hbm, woT_hbm,
            out_hbm,
            xaT, wqkv_v, wo_v, gate_v, mem0_v, wraw, woT_raw,
            wT_pad, woT_pad, QT, KA, VT, GT, PT, aT,
            W, WO, xb, mem_v, yb, outT, sems):
    def cp(src, dst, i):
        return pltpu.make_async_copy(src, dst, sems.at[i])

    c_xa = cp(xaT_hbm, xaT, 0)
    c_wqkv = cp(wqkv_hbm, wqkv_v, 1)
    c_wo = cp(wo_hbm, wo_v, 2)
    c_gate = cp(gate_hbm, gate_v, 3)
    c_mem = cp(mem0_hbm, mem0_v, 5)
    c_wq = cp(wq_hbm, wraw.at[0], 6)
    c_wk = cp(wk_hbm, wraw.at[1], 7)
    c_wv = cp(wv_hbm, wraw.at[2], 8)
    c_woT = cp(woT_hbm, woT_raw, 9)
    for c in (c_wqkv, c_gate, c_xa, c_wo, c_mem, c_woT, c_wq, c_wk, c_wv):
        c.start()

    c_wqkv.wait()
    c_gate.wait()
    wqkvT = wqkv_v[...].astype(F32).T
    zpad = jnp.zeros((DP - DHA, D), F32)
    for part in range(3):
        for h in range(HA):
            r0 = part * 448 + h * DHA
            blk = jnp.concatenate([wqkvT[r0:r0 + DHA, :], zpad], axis=0)
            if part == 0 and h == 0:
                rows = lax.broadcasted_iota(jnp.int32, (DP, D), 0)
                gw = jnp.broadcast_to(gate_v[...].astype(F32), (DP, D))
                blk = jnp.where(rows == 29, gw, blk)
            wT_pad[(part * HA + h) * DP:(part * HA + h + 1) * DP, :] = blk.astype(BF16)
    c_wo.wait()
    wo_f = wo_v[...].astype(F32)
    wo_rows = []
    for h in range(HA):
        wo_rows.append(wo_f[h * DHA:(h + 1) * DHA, :])
        wo_rows.append(zpad)
    wo_pad = jnp.concatenate(wo_rows, axis=0)
    woT_full = wo_pad.T.astype(BF16)
    for g in range(4):
        woT_pad[g] = _pk(woT_full[:, g * 128:(g + 1) * 128])

    c_xa.wait()
    qscale = (DHA ** -0.5) * LOG2E
    lane = lax.broadcasted_iota(jnp.int32, (WIN, 128), 1)
    for g in range(4):
        KA[g, 0:WIN // 2, :] = _pk(jnp.where(lane % DP == DHA, 1.0, 0.0).astype(BF16))
    VT[:, 0:WIN] = jnp.zeros((HA * DP // 2, WIN), U32)

    def wprep16(i, blk):
        w = jnp.swapaxes(wraw[i, pl.ds(pl.multiple_of(blk * 16, 16), 16)], 0, 1)
        for h in range(HB):
            for t in range(2):
                W[i * 32 + h * 2 + t, pl.ds(pl.multiple_of(blk * 8, 8), 8), :] = _pk(w[h][:, t * 128:(t + 1) * 128])

    def woprep(h):
        woh = woT_raw[h].T
        r0 = pl.multiple_of(h * 128, 128)
        for n in range(3):
            WO[n, pl.ds(r0, 128), :] = _pk(woh[:, n * 128:(n + 1) * 128])
        WO[3, pl.ds(r0, 128), :] = _pk(jnp.concatenate(
            [woh[:, 384:448], jnp.zeros((256, 64), BF16)], axis=1))

    def proj_body(b, carry, extra=None):
        c0 = pl.multiple_of(b * 128, 128)
        xt = xaT[:, pl.ds(c0, 128)]
        row = lax.broadcasted_iota(jnp.int32, (HA * DP, 128), 0) % DP
        qT = _dot(wT_pad[0:512, :], xt)
        kT = _dot(wT_pad[512:1024, :], xt)
        vT = _dot(wT_pad[1024:1536, :], xt)
        GT[:, pl.ds(c0, 128)] = qT[29:30, :]
        qT = jnp.where(row == DHA, NEG, qT * qscale)
        QT[:, pl.ds(c0, 128)] = _pk(qT.astype(BF16))
        k = kT.T.astype(BF16)
        for g in range(4):
            KA[g, pl.ds(pl.multiple_of(WIN // 2 + b * 64, 64), 64), :] = _pk(k[:, g * 128:(g + 1) * 128])
        vT = jnp.where(row == DHA, 1.0, vT)
        VT[:, pl.ds(pl.multiple_of(WIN + c0, 128), 128)] = _pk(vT.astype(BF16))
        xb[pl.ds(c0, 128), :] = xt.astype(F32).T
        aT[:, pl.ds(c0, 128)] = jnp.zeros((D, 128), F32)
        if extra is not None:
            extra(b)
        return carry

    def ex_wo(b):
        for j in range(4):
            woprep((b - 4) * 4 + j)

    def mk_ex_w(i, b0):
        def ex(b):
            for j in range(7):
                wprep16(i, (b - b0) * 7 + j)
        return ex

    lax.fori_loop(0, 4, proj_body, 0)
    c_woT.wait()
    lax.fori_loop(4, 8, functools.partial(proj_body, extra=ex_wo), 0)
    c_wq.wait()
    lax.fori_loop(8, 12, functools.partial(proj_body, extra=mk_ex_w(0, 8)), 0)
    c_wk.wait()
    lax.fori_loop(12, 16, functools.partial(proj_body, extra=mk_ex_w(1, 12)), 0)

    def a_scores(b, g, slot):
        c0 = pl.multiple_of(b * 128, 128)
        kk = lax.broadcasted_iota(jnp.int32, (128, 128), 0)
        qq = lax.broadcasted_iota(jnp.int32, (128, 128), 1)
        upper = kk > qq
        kw = _upk(KA[g, pl.ds(pl.multiple_of(b * 64, 64), 192), :])
        qg = QT[pl.ds(pl.multiple_of(g * 64, 64), 64), pl.ds(c0, 128)]
        for j in range(4):
            parts = []
            if j > 0:
                parts.append(jnp.zeros((j * 16, 128), U32))
            parts.append(qg[j * 16:(j + 1) * 16])
            if j < 3:
                parts.append(jnp.zeros(((3 - j) * 16, 128), U32))
            qm = _upk(_cat(parts))
            st = _dot(kw, qm)
            sm = jnp.where(upper, st[0:128], st[256:384])
            s1 = st[128:256]
            u = slot * 4 + j
            m = jnp.max(jnp.maximum(sm, s1), axis=0, keepdims=True)
            pm = jnp.exp2(sm - m)
            PT[u, 128:256, :] = jnp.exp2(s1 - m).astype(BF16)
            PT[u, 0:128, :] = jnp.where(upper, pm, 0.0).astype(BF16)
            PT[u, 256:384, :] = jnp.where(upper, 0.0, pm).astype(BF16)

    def a_pv(b, g, slot):
        c0 = pl.multiple_of(b * 128, 128)
        ots = []
        for j in range(4):
            vh = _upk(VT[pl.ds(pl.multiple_of(g * 64 + j * 16, 16), 16), pl.ds(c0, 384)])
            ot = _dot(vh, PT[slot * 4 + j])
            ot = ot * _recip(ot[DHA:DHA + 1, :])
            ots.append(ot.astype(BF16))
        return _cat(ots)

    def a_out(b, g, ot):
        c0 = pl.multiple_of(b * 128, 128)
        for r in range(4):
            w = _upk(woT_pad[g, r * 56:(r + 1) * 56, :])
            aT[r * 112:(r + 1) * 112, pl.ds(c0, 128)] += _dot(w, ot)

    c_mem.wait()
    mem_v[...] = mem0_v[...].astype(F32)
    c_wv.wait()
    if AFILL:
        a_scores(0, 0, 0)
        a_scores(0, 1, 1)
    for blk in range(28):
        wprep16(2, blk)

    def qkv_pass(lhs, fill=None):
        res = []
        for h in range(HB):
            res.append([[_dot(lhs, _upk(W[i * 32 + h * 2 + t])) for t in range(2)] for i in range(3)])
            if fill is not None:
                fill(h)
        return res

    def attention(qkv, valid, mid=None):
        scs = []
        for h in range(HB):
            q, k, v = qkv[h]
            scs.append(_dot_nt(q[0], k[0]) + _dot_nt(q[1], k[1]))
        if mid is not None:
            mid()
        ps = []
        rls = []
        for h in range(HB):
            sc = jnp.where(valid, scs[h] * (DHB ** -0.5 * LOG2E), NEG)
            m = jnp.max(sc, axis=1, keepdims=True)
            p = jnp.exp2(sc - m)
            ps.append(p.astype(BF16))
            rls.append(_recip(jnp.sum(p, axis=1, keepdims=True)))
        os_ = []
        for h in range(HB):
            v = qkv[h][2]
            os_.append(_dot(ps[h], v[0]) * rls[h])
            os_.append(_dot(ps[h], v[1]) * rls[h])
        return os_

    def o_pass(parts):
        acc = [None] * 4
        for c in range(8):
            lhs = jnp.concatenate(parts[4 * c:4 * c + 4], axis=1)
            for n in range(4):
                d = _dot(lhs, _upk(WO[n, c * 256:(c + 1) * 256, :]))
                acc[n] = d if acc[n] is None else acc[n] + d
        return jnp.concatenate(acc, axis=1)

    def pair_body(p, carry):
        qi = lax.broadcasted_iota(jnp.int32, (48, 48), 0)
        kj = lax.broadcasted_iota(jnp.int32, (48, 48), 1)
        validA = jnp.logical_and(kj < 40, jnp.logical_or(jnp.logical_or(kj >= 32, qi >= 32), kj <= qi))

        def pos(r):
            return jnp.where(r < 24, r + 8, r - 32)

        def ismem(r):
            return jnp.logical_and(r >= 24, r < 32)
        validB = jnp.logical_and(kj < 40, jnp.logical_or(jnp.logical_or(ismem(kj), ismem(qi)),
                                                         jnp.logical_or(pos(kj) <= pos(qi), qi >= 40)))
        r0 = pl.multiple_of(p * 64, 64)
        ab = p // 2
        ag = (p % 2) * 2
        pn = jnp.minimum(p + 1, 31)
        abn = pn // 2
        agn = (pn % 2) * 2

        def mk_fill(g, slot, gn):
            st = {}

            def fill(h):
                if AFILL and h == FILLH:
                    st['ot'] = a_pv(ab, g, slot)
                if AFILL and h == FILLH2:
                    a_out(ab, g, st['ot'])
                if AFILL and h == FILLH3:
                    a_scores(abn, gn, slot)
            return fill

        def mk_mid(g, slot):
            def mid():
                if AFILL and FILLH3 < 0:
                    a_scores(abn, g, slot)
            return mid

        lhsA = _cat([xb[pl.ds(r0, 32), :], mem_v[...], xb[pl.ds(r0 + 32, 8), :]]).astype(BF16)
        resA = qkv_pass(lhsA, mk_fill(ag, 0, agn))
        qkvA = [[[resA[h][i][t].astype(BF16) for t in range(2)] for i in range(3)] for h in range(HB)]
        oA = attention(qkvA, validA, mk_mid(agn, 0))
        olhsA = [_cat([o[0:24], o[32:40]]).astype(BF16) for o in oA]
        outA = o_pass(olhsA)
        yb[pl.ds(r0, 24), :] = outA[0:24]
        memA = outA[24:32, :D]

        lhsB = _cat([xb[pl.ds(r0 + 40, 24), :], memA]).astype(BF16)
        resB = qkv_pass(lhsB, mk_fill(ag + 1, 1, agn + 1))
        qkvB = [[[_cat([resB[h][i][t], resA[h][i][t][40:48], jnp.zeros((8, 128), F32)]).astype(BF16)
                  for t in range(2)] for i in range(3)] for h in range(HB)]
        oB = attention(qkvB, validB, mk_mid(agn + 1, 1))
        olhsB = [_cat([ob[0:40], oa[24:32]]).astype(BF16) for ob, oa in zip(oB, oA)]
        outB = o_pass(olhsB)
        yb[pl.ds(r0 + 40, 24), :] = outB[0:24]
        mem_v[...] = outB[24:32, :D]
        yb[pl.ds(r0 + 32, 8), :] = outB[32:40]
        yb[pl.ds(r0 + 24, 8), :] = outB[40:48]
        return carry

    lax.fori_loop(0, NSEG // 2, pair_body, 0)

    def fin_body(b, carry):
        c0 = pl.multiple_of(b * 128, 128)
        bT = yb[pl.ds(c0, 128), :].T[:D, :]
        g = jax.nn.sigmoid(GT[:, pl.ds(c0, 128)])
        outT[:, pl.ds(c0, 128)] = (g * aT[:, pl.ds(c0, 128)] + (1.0 - g) * bT).astype(BF16)
        return carry
    lax.fori_loop(0, S // 128, fin_body, 0)

    c_out = cp(outT, out_hbm, 10)
    c_out.start()
    c_out.wait()


@jax.jit
def pallas_gated_mix__sliding_block__memory_aug_recurrent_mem_tr__prompt_kernel(
        A_x, A_wqkv, A_wo, B_x, B_mem0, B_Wq, B_Wk, B_Wv, B_Wo, B_seg_len, gate_w):
    xaT = A_x[0].T
    mem0 = B_mem0[0]
    woT = B_Wo.transpose(0, 2, 1)
    gate = gate_w.reshape(1, D)
    any_spec = pl.BlockSpec(memory_space=pl.ANY)
    scratch = [
        pltpu.VMEM((D, S), BF16),
        pltpu.VMEM((D, 3 * D), BF16),
        pltpu.VMEM((D, D), BF16),
        pltpu.VMEM((1, D), BF16),
        pltpu.VMEM((MEM, D), BF16),
        pltpu.VMEM((3, D, HB, DHB), BF16),
        pltpu.VMEM((HB, D, DHB), BF16),
        pltpu.VMEM((3 * 512, D), BF16),
        pltpu.VMEM((4, D // 2, 128), U32),
        pltpu.VMEM((256, S), U32),
        pltpu.VMEM((4, (WIN + S) // 2, 128), U32),
        pltpu.VMEM((256, WIN + S), U32),
        pltpu.VMEM((1, S), F32),
        pltpu.VMEM((8, 384, 128), BF16),
        pltpu.VMEM((D, S), F32),
        pltpu.VMEM((96, D // 2, 128), U32),
        pltpu.VMEM((4, HB * DHB // 2, 128), U32),
        pltpu.VMEM((S, D), F32),
        pltpu.VMEM((MEM, D), F32),
        pltpu.VMEM((S, 512), F32),
        pltpu.VMEM((D, S), BF16),
        pltpu.SemaphoreType.DMA((11,)),
    ]
    outT = pl.pallas_call(
        _kernel,
        out_shape=jax.ShapeDtypeStruct((D, S), BF16),
        in_specs=[any_spec] * 9,
        out_specs=any_spec,
        scratch_shapes=scratch,
        compiler_params=pltpu.CompilerParams(vmem_limit_bytes=110 * 1024 * 1024),
    )(xaT, A_wqkv, A_wo, gate, mem0, B_Wq, B_Wk, B_Wv, woT)
    return outT.T[None]
```

```python
import functools
import jax
import jax.numpy as jnp
from jax import lax
import jax.experimental.pallas as pl
import jax.experimental.pallas.tpu as pltpu

F32 = jnp.float32
BF16 = jnp.bfloat16
U32 = jnp.uint32

S = 2048
D = 448
HA = 16
DHA = 28
DP = 32
WIN = 256
HB = 16
DHB = 256
MEM = 8
SEG = 32
NBLK = S // 128
NEG = -1e30
LOG2E = 1.4426950408889634
FILLH = -1
FILLH2 = 4
SH = [8, 10, 12, 14]
SPLIT = 1
FINH = 7
FINS = 1


def _dot(a, b):
    return jnp.dot(a, b, preferred_element_type=F32)


def _dot_nt(a, b):
    return lax.dot_general(a, b, (((1,), (1,)), ((), ())), preferred_element_type=F32)


def _pk(x):
    return pltpu.bitcast(x, U32)


def _upk(x):
    return pltpu.bitcast(x, BF16)


def _recip(x):
    r = pl.reciprocal(x, approx=True)
    return r * (2.0 - x * r)


def _cat(parts):
    return jnp.concatenate(parts, axis=0)


def _kernel(xT_hbm, wqkv_hbm, wo_hbm, gate_hbm, mem0_hbm, wq_hbm, wk_hbm, wv_hbm, woT_hbm,
            out_hbm,
            xT, wqkv_v, wo_v, gate_v, mem0_v, wraw, woT_raw,
            wT_pad, woT_pad, QT, KA, VT, GT, PT, aT,
            W, WO, xb, mem_v, yb, outT, sems):
    def cp(src, dst, i):
        return pltpu.make_async_copy(src, dst, sems.at[i])

    c_x = cp(xT_hbm, xT, 0)
    c_wqkv = cp(wqkv_hbm, wqkv_v, 1)
    c_wo = cp(wo_hbm, wo_v, 2)
    c_gate = cp(gate_hbm, gate_v, 3)
    c_mem = cp(mem0_hbm, mem0_v, 4)
    c_wq = cp(wq_hbm, wraw.at[0], 5)
    c_wk = cp(wk_hbm, wraw.at[1], 6)
    c_wv = cp(wv_hbm, wraw.at[2], 7)
    c_woT = cp(woT_hbm, woT_raw, 8)
    for c in (c_wqkv, c_gate, c_x, c_wo, c_mem, c_woT, c_wq, c_wk, c_wv):
        c.start()

    c_wqkv.wait()
    c_gate.wait()
    wqkvT = wqkv_v[...].astype(F32).T
    zpad = jnp.zeros((DP - DHA, D), F32)
    for part in range(3):
        for h in range(HA):
            r0 = part * 448 + h * DHA
            blk = _cat([wqkvT[r0:r0 + DHA, :], zpad])
            if part == 0 and h == 0:
                rows = lax.broadcasted_iota(jnp.int32, (DP, D), 0)
                gw = jnp.broadcast_to(gate_v[...].astype(F32), (DP, D))
                blk = jnp.where(rows == 29, gw, blk)
            wT_pad[(part * HA + h) * DP:(part * HA + h + 1) * DP, :] = blk.astype(BF16)
    c_wo.wait()
    wo_f = wo_v[...].astype(F32)
    wo_rows = []
    for h in range(HA):
        wo_rows.append(wo_f[h * DHA:(h + 1) * DHA, :])
        wo_rows.append(zpad)
    woT_full = _cat(wo_rows).T.astype(BF16)
    for g in range(4):
        woT_pad[g] = _pk(woT_full[:, g * 128:(g + 1) * 128])

    c_x.wait()
    qscale = (DHA ** -0.5) * LOG2E
    lane = lax.broadcasted_iota(jnp.int32, (WIN, 128), 1)
    for g in range(4):
        KA[g, 0:WIN // 2, :] = _pk(jnp.where(lane % DP == DHA, 1.0, 0.0).astype(BF16))
    VT[:, 0:WIN] = jnp.zeros((HA * DP // 2, WIN), U32)

    def wprep16(i, blk):
        w = jnp.swapaxes(wraw[i, pl.ds(pl.multiple_of(blk * 16, 16), 16)], 0, 1)
        for h in range(HB):
            for t in range(2):
                W[i * 32 + h * 2 + t, pl.ds(pl.multiple_of(blk * 8, 8), 8), :] = _pk(w[h][:, t * 128:(t + 1) * 128])

    def woprep(h):
        woh = woT_raw[h].T
        r0 = pl.multiple_of(h * 128, 128)
        for n in range(3):
            WO[n, pl.ds(r0, 128), :] = _pk(woh[:, n * 128:(n + 1) * 128])
        WO[3, pl.ds(r0, 128), :] = _pk(jnp.concatenate(
            [woh[:, 384:448], jnp.zeros((256, 64), BF16)], axis=1))

    def proj_body(b, carry, extra=None):
        c0 = pl.multiple_of(b * 128, 128)
        xt = xT[:, pl.ds(c0, 128)]
        row = lax.broadcasted_iota(jnp.int32, (HA * DP, 128), 0) % DP
        qT = _dot(wT_pad[0:512, :], xt)
        kT = _dot(wT_pad[512:1024, :], xt)
        vT = _dot(wT_pad[1024:1536, :], xt)
        GT[:, pl.ds(c0, 128)] = qT[29:30, :]
        qT = jnp.where(row == DHA, NEG, qT * qscale)
        QT[:, pl.ds(c0, 128)] = _pk(qT.astype(BF16))
        k = kT.T.astype(BF16)
        for g in range(4):
            KA[g, pl.ds(pl.multiple_of(WIN // 2 + b * 64, 64), 64), :] = _pk(k[:, g * 128:(g + 1) * 128])
        vT = jnp.where(row == DHA, 1.0, vT)
        VT[:, pl.ds(pl.multiple_of(WIN + c0, 128), 128)] = _pk(vT.astype(BF16))
        xb[pl.ds(c0, 128), :] = xt.astype(F32).T
        aT[:, pl.ds(c0, 128)] = jnp.zeros((D, 128), F32)
        yb[pl.ds(c0, 128), :] = jnp.zeros((128, 512), BF16)
        if extra is not None:
            extra(b)
        return carry

    def ex_wo(b):
        for j in range(4):
            woprep((b - 4) * 4 + j)

    def mk_ex_w(i, b0):
        def ex(b):
            for j in range(7):
                wprep16(i, (b - b0) * 7 + j)
        return ex

    lax.fori_loop(0, 4, proj_body, 0)
    c_woT.wait()
    lax.fori_loop(4, 8, functools.partial(proj_body, extra=ex_wo), 0)
    c_wq.wait()
    lax.fori_loop(8, 12, functools.partial(proj_body, extra=mk_ex_w(0, 8)), 0)
    c_wk.wait()
    lax.fori_loop(12, 16, functools.partial(proj_body, extra=mk_ex_w(1, 12)), 0)

    def a_scores(b, g, slot, units=(0, 1, 2, 3)):
        c0 = pl.multiple_of(b * 128, 128)
        kk = lax.broadcasted_iota(jnp.int32, (128, 128), 0)
        qq = lax.broadcasted_iota(jnp.int32, (128, 128), 1)
        upper = kk > qq
        for j in units:
            qj = QT[pl.ds(pl.multiple_of(g * 64 + j * 16, 16), 16), pl.ds(c0, 128)]
            parts = []
            if j > 0:
                parts.append(jnp.zeros((j * 16, 128), U32))
            parts.append(qj)
            if j < 3:
                parts.append(jnp.zeros(((3 - j) * 16, 128), U32))
            qm = _upk(_cat(parts))
            if SPLIT:
                st = _cat([_dot(_upk(KA[g, pl.ds(pl.multiple_of(b * 64 + r * 48, 16), 48), :]), qm) for r in range(4)])
            else:
                st = _dot(_upk(KA[g, pl.ds(pl.multiple_of(b * 64, 64), 192), :]), qm)
            sm = jnp.where(upper, st[0:128], st[256:384])
            s1 = st[128:256]
            u = slot * 4 + j
            m = jnp.max(jnp.maximum(sm, s1), axis=0, keepdims=True)
            pm = jnp.exp2(sm - m)
            PT[u, 128:256, :] = jnp.exp2(s1 - m).astype(BF16)
            PT[u, 0:128, :] = jnp.where(upper, pm, 0.0).astype(BF16)
            PT[u, 256:384, :] = jnp.where(upper, 0.0, pm).astype(BF16)

    def a_pv(b, g, slot):
        c0 = pl.multiple_of(b * 128, 128)
        ots = []
        for j in range(4):
            vh = _upk(VT[pl.ds(pl.multiple_of(g * 64 + j * 16, 16), 16), pl.ds(c0, 384)])
            ot = _dot(vh, PT[slot * 4 + j])
            ot = ot * _recip(ot[DHA:DHA + 1, :])
            ots.append(ot.astype(BF16))
        return _cat(ots)

    def a_out(b, g, ot):
        c0 = pl.multiple_of(b * 128, 128)
        for r in range(4):
            w = _upk(woT_pad[g, r * 56:(r + 1) * 56, :])
            aT[r * 112:(r + 1) * 112, pl.ds(c0, 128)] += _dot(w, ot)

    c_mem.wait()
    mem_v[...] = mem0_v[...].astype(F32)
    c_wv.wait()
    a_scores(0, 0, 0)
    a_scores(0, 1, 1)
    for blk in range(28):
        wprep16(2, blk)

    def qkv_pass(lhs, fill):
        res = []
        fill(-1)
        for h in range(HB):
            res.append([[_dot(lhs, _upk(W[i * 32 + h * 2 + t])) for t in range(2)] for i in range(3)])
            fill(h)
        return res

    def attention(qkv, valid):
        scs = []
        for h in range(HB):
            q, k, v = qkv[h]
            scs.append(_dot_nt(q[0], k[0]) + _dot_nt(q[1], k[1]))
        ps = []
        rls = []
        for h in range(HB):
            sc = jnp.where(valid, scs[h] * (DHB ** -0.5 * LOG2E), NEG)
            m = jnp.max(sc, axis=1, keepdims=True)
            p = jnp.exp2(sc - m)
            ps.append(p.astype(BF16))
            rls.append(_recip(jnp.sum(p, axis=1, keepdims=True)))
        os_ = []
        for h in range(HB):
            v = qkv[h][2]
            os_.append(_dot(ps[h], v[0]) * rls[h])
            os_.append(_dot(ps[h], v[1]) * rls[h])
        return os_

    def o_pass(parts):
        acc = [None] * 4
        for c in range(8):
            lhs = jnp.concatenate(parts[4 * c:4 * c + 4], axis=1)
            for n in range(4):
                d = _dot(lhs, _upk(WO[n, c * 256:(c + 1) * 256, :]))
                acc[n] = d if acc[n] is None else acc[n] + d
        return jnp.concatenate(acc, axis=1)

    def fin(b):
        c0 = pl.multiple_of(b * 128, 128)
        bT = yb[pl.ds(c0, 128), :].T[:D, :].astype(F32)
        g = jax.nn.sigmoid(GT[:, pl.ds(c0, 128)])
        outT[:, pl.ds(c0, 128)] = (g * aT[:, pl.ds(c0, 128)] + (1.0 - g) * bT).astype(BF16)

    def out_copy(b):
        c0 = pl.multiple_of(b * 128, 128)
        return pltpu.make_async_copy(outT.at[:, pl.ds(c0, 128)], out_hbm.at[:, pl.ds(c0, 128)], sems.at[9])

    def pair_body(p, extra=None):
        qi = lax.broadcasted_iota(jnp.int32, (48, 48), 0)
        kj = lax.broadcasted_iota(jnp.int32, (48, 48), 1)
        validA = jnp.logical_and(kj < 40, jnp.logical_or(jnp.logical_or(kj >= 32, qi >= 32), kj <= qi))

        def pos(r):
            return jnp.where(r < 24, r + 8, r - 32)

        def ismem(r):
            return jnp.logical_and(r >= 24, r < 32)
        validB = jnp.logical_and(kj < 40, jnp.logical_or(jnp.logical_or(ismem(kj), ismem(qi)),
                                                         jnp.logical_or(pos(kj) <= pos(qi), qi >= 40)))
        r0 = pl.multiple_of(p * 64, 64)
        ab = p // 2
        ag = (p % 2) * 2
        pn = jnp.minimum(p + 1, 31)
        abn = pn // 2
        agn = (pn % 2) * 2

        def mk_fill(g, slot, gn):
            st = {}

            def fill(h):
                if h == FILLH:
                    st['ot'] = a_pv(ab, g, slot)
                if h == FILLH2:
                    a_out(ab, g, st['ot'])
                if h in SH:
                    a_scores(abn, gn, slot, units=(SH.index(h),))
                if h == FINH and slot == FINS and extra is not None:
                    extra()
            return fill

        lhsA = _cat([xb[pl.ds(r0, 32), :], mem_v[...], xb[pl.ds(r0 + 32, 8), :]]).astype(BF16)
        resA = qkv_pass(lhsA, mk_fill(ag, 0, agn))
        qkvA = [[[resA[h][i][t].astype(BF16) for t in range(2)] for i in range(3)] for h in range(HB)]
        oA = attention(qkvA, validA)
        olhsA = [_cat([o[0:24], o[32:40]]).astype(BF16) for o in oA]
        outA = o_pass(olhsA)
        memA = outA[24:32, :D]

        lhsB = _cat([xb[pl.ds(r0 + 40, 24), :], memA]).astype(BF16)
        resB = qkv_pass(lhsB, mk_fill(ag + 1, 1, agn + 1))
        qkvB = [[[_cat([resB[h][i][t], resA[h][i][t][40:48], jnp.zeros((8, 128), F32)]).astype(BF16)
                  for t in range(2)] for i in range(3)] for h in range(HB)]
        oB = attention(qkvB, validB)
        olhsB = [_cat([ob[0:40], oa[24:32]]).astype(BF16) for ob, oa in zip(oB, oA)]
        outB = o_pass(olhsB)
        mem_v[...] = outB[24:32, :D]
        yb[pl.ds(r0, 64), :] = _cat([outA[0:24], outB[40:48], outB[32:40], outB[0:24]]).astype(BF16)

    def block_body(b, carry):
        bp = (b + NBLK - 1) % NBLK

        def extra():
            fin(bp)
            out_copy(bp).start()
        pair_body(2 * b, extra)
        pair_body(2 * b + 1)
        return carry

    lax.fori_loop(0, NBLK, block_body, 0)
    for b in range(NBLK):
        out_copy(b).wait()
    fin(NBLK - 1)
    out_copy(NBLK - 1).start()
    out_copy(NBLK - 1).wait()


@jax.jit
def pallas_gated_mix__sliding_block__memory_aug_recurrent_mem_tr__prompt_kernel(
        A_x, A_wqkv, A_wo, B_x, B_mem0, B_Wq, B_Wk, B_Wv, B_Wo, B_seg_len, gate_w):
    xT = A_x[0].T
    mem0 = B_mem0[0]
    woT = B_Wo.transpose(0, 2, 1)
    gate = gate_w.reshape(1, D)
    any_spec = pl.BlockSpec(memory_space=pl.ANY)
    scratch = [
        pltpu.VMEM((D, S), BF16),
        pltpu.VMEM((D, 3 * D), BF16),
        pltpu.VMEM((D, D), BF16),
        pltpu.VMEM((1, D), BF16),
        pltpu.VMEM((MEM, D), BF16),
        pltpu.VMEM((3, D, HB, DHB), BF16),
        pltpu.VMEM((HB, D, DHB), BF16),
        pltpu.VMEM((3 * 512, D), BF16),
        pltpu.VMEM((4, D // 2, 128), U32),
        pltpu.VMEM((256, S), U32),
        pltpu.VMEM((4, (WIN + S) // 2, 128), U32),
        pltpu.VMEM((256, WIN + S), U32),
        pltpu.VMEM((1, S), F32),
        pltpu.VMEM((8, 384, 128), BF16),
        pltpu.VMEM((D, S), F32),
        pltpu.VMEM((96, D // 2, 128), U32),
        pltpu.VMEM((4, HB * DHB // 2, 128), U32),
        pltpu.VMEM((S, D), F32),
        pltpu.VMEM((MEM, D), F32),
        pltpu.VMEM((S, 512), BF16),
        pltpu.VMEM((D, S), BF16),
        pltpu.SemaphoreType.DMA((10,)),
    ]
    outT = pl.pallas_call(
        _kernel,
        out_shape=jax.ShapeDtypeStruct((D, S), BF16),
        in_specs=[any_spec] * 9,
        out_specs=any_spec,
        scratch_shapes=scratch,
        compiler_params=pltpu.CompilerParams(vmem_limit_bytes=110 * 1024 * 1024),
    )(xT, A_wqkv, A_wo, gate, mem0, B_Wq, B_Wk, B_Wv, woT)
    return outT.T[None]
```

```python
import functools
import jax
import jax.numpy as jnp
from jax import lax
import jax.experimental.pallas as pl
import jax.experimental.pallas.tpu as pltpu

F32 = jnp.float32
BF16 = jnp.bfloat16
U32 = jnp.uint32

S = 2048
D = 448
HA = 16
DHA = 28
DP = 32
WIN = 256
HB = 16
DHB = 256
MEM = 8
NBLK = S // 128
NPAIR = S // 64
NEG = -1e30
LOG2E = 1.4426950408889634

PV_AT = (-1, -1)
OUT_AT = (16, 4)
SCORES_AT = ((5, 8, 11, 14), (8, 10, 12, 14))
FIN_AT = 7


def _dot(a, b):
    return jnp.dot(a, b, preferred_element_type=F32)


def _dot_nt(a, b):
    return lax.dot_general(a, b, (((1,), (1,)), ((), ())), preferred_element_type=F32)


def _pk(x):
    return pltpu.bitcast(x, U32)


def _upk(x):
    return pltpu.bitcast(x, BF16)


def _recip(x):
    r = pl.reciprocal(x, approx=True)
    return r * (2.0 - x * r)


def _cat(parts):
    return jnp.concatenate(parts, axis=0)


def _iota(shape, d):
    return lax.broadcasted_iota(jnp.int32, shape, d)


def _kernel(xT_hbm, wqkv_hbm, wo_hbm, gate_hbm, mem0_hbm, wq_hbm, wk_hbm, wv_hbm, woT_hbm,
            out_hbm,
            xT, wqkv_v, wo_v, gate_v, mem0_v, wraw, woT_raw,
            wT_pad, woT_pad, QT, KA, VT, GT, PT, aT,
            W, WO, xb, mem_v, yb, OC, outT, sems):
    def cp(src, dst, i):
        return pltpu.make_async_copy(src, dst, sems.at[i])

    c_x = cp(xT_hbm, xT, 0)
    c_wqkv = cp(wqkv_hbm, wqkv_v, 1)
    c_wo = cp(wo_hbm, wo_v, 2)
    c_gate = cp(gate_hbm, gate_v, 3)
    c_mem = cp(mem0_hbm, mem0_v, 4)
    c_wq = cp(wq_hbm, wraw.at[0], 5)
    c_wk = cp(wk_hbm, wraw.at[1], 6)
    c_wv = cp(wv_hbm, wraw.at[2], 7)
    c_woT = cp(woT_hbm, woT_raw, 8)
    for c in (c_wqkv, c_gate, c_x, c_wo, c_mem, c_woT, c_wq, c_wk, c_wv):
        c.start()

    c_wqkv.wait()
    c_gate.wait()
    wqkvT = wqkv_v[...].astype(F32).T
    zpad = jnp.zeros((DP - DHA, D), F32)
    for part in range(3):
        for h in range(HA):
            r0 = part * D + h * DHA
            blk = _cat([wqkvT[r0:r0 + DHA, :], zpad])
            if part == 0 and h == 0:
                gw = jnp.broadcast_to(gate_v[...].astype(F32), (DP, D))
                blk = jnp.where(_iota((DP, D), 0) == 29, gw, blk)
            wT_pad[(part * HA + h) * DP:(part * HA + h + 1) * DP, :] = blk.astype(BF16)
    c_wo.wait()
    wo_f = wo_v[...].astype(F32)
    wo_rows = []
    for h in range(HA):
        wo_rows.append(wo_f[h * DHA:(h + 1) * DHA, :])
        wo_rows.append(zpad)
    woT_full = _cat(wo_rows).T.astype(BF16)
    for g in range(4):
        woT_pad[g] = _pk(woT_full[:, g * 128:(g + 1) * 128])

    c_x.wait()
    qscale = (DHA ** -0.5) * LOG2E
    for g in range(4):
        KA[g, 0:WIN // 2, :] = _pk(jnp.where(_iota((WIN, 128), 1) % DP == DHA, 1.0, 0.0).astype(BF16))
    VT[:, 0:WIN] = jnp.zeros((HA * DP // 2, WIN), U32)

    def wprep16(i, blk):
        w = jnp.swapaxes(wraw[i, pl.ds(pl.multiple_of(blk * 16, 16), 16)], 0, 1)
        for h in range(HB):
            for t in range(2):
                W[i * 32 + h * 2 + t, pl.ds(pl.multiple_of(blk * 8, 8), 8), :] = _pk(w[h][:, t * 128:(t + 1) * 128])

    def woprep(h):
        woh = woT_raw[h].T
        r0 = pl.multiple_of(h * 128, 128)
        for n in range(3):
            WO[n, pl.ds(r0, 128), :] = _pk(woh[:, n * 128:(n + 1) * 128])
        WO[3, pl.ds(r0, 128), :] = _pk(jnp.concatenate(
            [woh[:, 384:448], jnp.zeros((256, 64), BF16)], axis=1))

    def proj_body(b, carry, extra=None):
        c0 = pl.multiple_of(b * 128, 128)
        xt = xT[:, pl.ds(c0, 128)]
        row = _iota((HA * DP, 128), 0) % DP
        qT = _dot(wT_pad[0:512, :], xt)
        kT = _dot(wT_pad[512:1024, :], xt)
        vT = _dot(wT_pad[1024:1536, :], xt)
        GT[:, pl.ds(c0, 128)] = qT[29:30, :]
        qT = jnp.where(row == DHA, NEG, qT * qscale)
        QT[:, pl.ds(c0, 128)] = _pk(qT.astype(BF16))
        k = kT.T.astype(BF16)
        for g in range(4):
            KA[g, pl.ds(pl.multiple_of(WIN // 2 + b * 64, 64), 64), :] = _pk(k[:, g * 128:(g + 1) * 128])
        vT = jnp.where(row == DHA, 1.0, vT)
        VT[:, pl.ds(pl.multiple_of(WIN + c0, 128), 128)] = _pk(vT.astype(BF16))
        xb[pl.ds(c0, 128), :] = xt.astype(F32).T
        aT[:, pl.ds(c0, 128)] = jnp.zeros((D, 128), F32)
        yb[pl.ds(pl.multiple_of(16 + c0, 16), 128), :] = jnp.zeros((128, 512), BF16)
        if extra is not None:
            extra(b)
        return carry

    def ex_wo(b):
        for j in range(4):
            woprep((b - 4) * 4 + j)

    def mk_ex_w(i, b0):
        def ex(b):
            for j in range(7):
                wprep16(i, (b - b0) * 7 + j)
        return ex

    lax.fori_loop(0, 4, proj_body, 0)
    c_woT.wait()
    lax.fori_loop(4, 8, functools.partial(proj_body, extra=ex_wo), 0)
    c_wq.wait()
    lax.fori_loop(8, 12, functools.partial(proj_body, extra=mk_ex_w(0, 8)), 0)
    c_wk.wait()
    lax.fori_loop(12, 16, functools.partial(proj_body, extra=mk_ex_w(1, 12)), 0)

    def a_scores(b, g, slot, units=(0, 1, 2, 3)):
        c0 = pl.multiple_of(b * 128, 128)
        upper = _iota((128, 128), 0) > _iota((128, 128), 1)
        for j in units:
            qj = QT[pl.ds(pl.multiple_of(g * 64 + j * 16, 16), 16), pl.ds(c0, 128)]
            parts = []
            if j > 0:
                parts.append(jnp.zeros((j * 16, 128), U32))
            parts.append(qj)
            if j < 3:
                parts.append(jnp.zeros(((3 - j) * 16, 128), U32))
            qm = _upk(_cat(parts))
            st = _cat([_dot(_upk(KA[g, pl.ds(pl.multiple_of(b * 64 + r * 48, 16), 48), :]), qm)
                       for r in range(4)])
            sm = jnp.where(upper, st[0:128], st[256:384])
            s1 = st[128:256]
            u = slot * 4 + j
            m = jnp.max(jnp.maximum(sm, s1), axis=0, keepdims=True)
            pm = jnp.exp2(sm - m)
            PT[u, 128:256, :] = jnp.exp2(s1 - m).astype(BF16)
            PT[u, 0:128, :] = jnp.where(upper, pm, 0.0).astype(BF16)
            PT[u, 256:384, :] = jnp.where(upper, 0.0, pm).astype(BF16)

    def a_pv(b, g, slot):
        c0 = pl.multiple_of(b * 128, 128)
        ots = []
        for j in range(4):
            vh = _upk(VT[pl.ds(pl.multiple_of(g * 64 + j * 16, 16), 16), pl.ds(c0, 384)])
            ot = _dot(vh, PT[slot * 4 + j])
            ot = ot * _recip(ot[DHA:DHA + 1, :])
            ots.append(ot.astype(BF16))
        return _cat(ots)

    def a_out(b, g, ot):
        c0 = pl.multiple_of(b * 128, 128)
        for r in range(4):
            w = _upk(woT_pad[g, r * 56:(r + 1) * 56, :])
            aT[r * 112:(r + 1) * 112, pl.ds(c0, 128)] += _dot(w, ot)

    c_mem.wait()
    mem_v[...] = mem0_v[...].astype(F32)
    c_wv.wait()
    a_scores(0, 0, 0)
    a_scores(0, 1, 1)
    for blk in range(28):
        wprep16(2, blk)

    def qkv_pass(lhs, fill):
        res = []
        fill(-1)
        for h in range(HB):
            res.append([[_dot(lhs, _upk(W[i * 32 + h * 2 + t])) for t in range(2)] for i in range(3)])
            fill(h)
        return res

    def scores(q, k):
        return [_dot_nt(q[h][0], k[h][0]) + _dot_nt(q[h][1], k[h][1]) for h in range(HB)]

    def softmax(scs, valid):
        ps, rls = [], []
        for sc in scs:
            sc = jnp.where(valid, sc * (DHB ** -0.5 * LOG2E), NEG)
            m = jnp.max(sc, axis=1, keepdims=True)
            p = jnp.exp2(sc - m)
            ps.append(p.astype(BF16))
            rls.append(_recip(jnp.sum(p, axis=1, keepdims=True)))
        return ps, rls

    def pv(ps, rls, v):
        return [_dot(ps[h], v[h][t]) * rls[h] for h in range(HB) for t in range(2)]

    def o_pass(parts):
        acc = [None] * 4
        for c in range(8):
            lhs = jnp.concatenate(parts[4 * c:4 * c + 4], axis=1)
            for n in range(4):
                d = _dot(lhs, _upk(WO[n, c * 256:(c + 1) * 256, :]))
                acc[n] = d if acc[n] is None else acc[n] + d
        return jnp.concatenate(acc, axis=1)

    def fin(b):
        c0 = pl.multiple_of(b * 128, 128)
        bT = yb[pl.ds(pl.multiple_of(16 + c0, 16), 128), :].T[:D, :].astype(F32)
        g = jax.nn.sigmoid(GT[:, pl.ds(c0, 128)])
        outT[:, pl.ds(c0, 128)] = (g * aT[:, pl.ds(c0, 128)] + (1.0 - g) * bT).astype(BF16)

    def out_copy(b):
        c0 = pl.multiple_of(b * 128, 128)
        return pltpu.make_async_copy(outT.at[:, pl.ds(c0, 128)], out_hbm.at[:, pl.ds(c0, 128)], sems.at[9])

    def pair_body(p, carry_o, extra=None):
        i16, j48 = _iota((16, 48), 0), _iota((16, 48), 1)
        validA = (j48 < 40) & ((i16 < 8) | (j48 >= 32) | (j48 <= i16 - 8))
        i64, j80 = _iota((64, 80), 0), _iota((64, 80), 1)
        isA = (i64 >= 16) & (i64 < 40)
        posB = jnp.where(i64 < 8, 31, jnp.where(i64 < 16, i64 - 8, i64 - 32))
        validB = ((isA & (((j80 < 32) & (j80 <= i64 - 8)) | ((j80 >= 32) & (j80 < 40))))
                  | (jnp.logical_not(isA) & (((j80 >= 40) & (j80 < 72) & (j80 - 40 <= posB)) | (j80 >= 72))))
        r0 = pl.multiple_of(p * 64, 64)
        ab = p // 2
        ag = (p % 2) * 2
        pn = jnp.minimum(p + 1, NPAIR - 1)
        abn = pn // 2
        agn = (pn % 2) * 2

        def mk_fill(g, slot, gn):
            st = {}

            def fill(h):
                if h == PV_AT[slot]:
                    st['ot'] = a_pv(ab, g, slot)
                if h == OUT_AT[slot]:
                    a_out(ab, g, st['ot'])
                if h in SCORES_AT[slot]:
                    a_scores(abn, gn, slot, units=(SCORES_AT[slot].index(h),))
                if h == FIN_AT and slot == 1 and extra is not None:
                    extra()
            return fill

        def per(fn):
            return [[fn(h, t) for t in range(2)] for h in range(HB)]

        fillA = mk_fill(ag, 0, agn)
        lhsA = _cat([xb[pl.ds(r0, 32), :], mem_v[...], xb[pl.ds(r0 + 32, 8), :]]).astype(BF16)
        resA = qkv_pass(lhsA, fillA)
        kA = per(lambda h, t: resA[h][1][t].astype(BF16))
        vA = per(lambda h, t: resA[h][2][t].astype(BF16))
        qA = per(lambda h, t: _cat([resA[h][0][t][32:40], resA[h][0][t][0:8]]).astype(BF16))
        scA = scores(qA, kA)
        fillA(HB)
        oA = pv(*softmax(scA, validA), vA)
        outA = o_pass([_cat([oA[n], carry_o[n]]).astype(BF16) for n in range(32)])
        memA = outA[0:8, :D]
        yb[pl.ds(pl.multiple_of(16 + r0, 8), 8), :] = outA[8:16].astype(BF16)
        yb[pl.ds(r0, 16), :] = outA[16:32].astype(BF16)

        fillB = mk_fill(ag + 1, 1, agn + 1)
        lhsB = _cat([xb[pl.ds(r0 + 40, 24), :], memA]).astype(BF16)
        resB = qkv_pass(lhsB, fillB)
        kB = per(lambda h, t: resB[h][1][t].astype(BF16))
        vB = per(lambda h, t: resB[h][2][t].astype(BF16))
        qB = per(lambda h, t: _cat([resB[h][0][t][24:32], resA[h][0][t][40:48],
                                    resA[h][0][t][8:32], resB[h][0][t][0:24]]).astype(BF16))
        kD = per(lambda h, t: _cat([kA[h][t], kB[h][t]]))
        vD = per(lambda h, t: _cat([vA[h][t], vB[h][t]]))
        scB = scores(qB, kD)
        oB = pv(*softmax(scB, validB), vD)
        outB = o_pass([o[0:48].astype(BF16) for o in oB])
        mem_v[...] = outB[0:8, :D]
        yb[pl.ds(pl.multiple_of(16 + r0 + 8, 8), 24), :] = outB[16:40].astype(BF16)
        yb[pl.ds(pl.multiple_of(16 + r0 + 32, 16), 16), :] = _cat([outB[8:16], outB[40:48]]).astype(BF16)
        return [o[48:64] for o in oB]

    def block_body(b, carry):
        bp = (b + NBLK - 1) % NBLK

        def extra():
            fin(bp)
            out_copy(bp).start()
        co = [OC[n] for n in range(32)]
        co = pair_body(2 * b, co, extra)
        co = pair_body(2 * b + 1, co)
        for n in range(32):
            OC[n] = co[n]
        return carry

    OC[...] = jnp.zeros((32, 16, 128), F32)
    lax.fori_loop(0, NBLK, block_body, 0)
    out_last = o_pass([OC[n].astype(BF16) for n in range(32)])
    yb[S:S + 16, :] = out_last.astype(BF16)
    for b in range(NBLK):
        out_copy(b).wait()
    fin(NBLK - 1)
    out_copy(NBLK - 1).start()
    out_copy(NBLK - 1).wait()


@jax.jit
def pallas_gated_mix__sliding_block__memory_aug_recurrent_mem_tr__prompt_kernel(
        A_x, A_wqkv, A_wo, B_x, B_mem0, B_Wq, B_Wk, B_Wv, B_Wo, B_seg_len, gate_w):
    xT = A_x[0].T
    mem0 = B_mem0[0]
    woT = B_Wo.transpose(0, 2, 1)
    gate = gate_w.reshape(1, D)
    any_spec = pl.BlockSpec(memory_space=pl.ANY)
    scratch = [
        pltpu.VMEM((D, S), BF16),
        pltpu.VMEM((D, 3 * D), BF16),
        pltpu.VMEM((D, D), BF16),
        pltpu.VMEM((1, D), BF16),
        pltpu.VMEM((MEM, D), BF16),
        pltpu.VMEM((3, D, HB, DHB), BF16),
        pltpu.VMEM((HB, D, DHB), BF16),
        pltpu.VMEM((3 * 512, D), BF16),
        pltpu.VMEM((4, D // 2, 128), U32),
        pltpu.VMEM((256, S), U32),
        pltpu.VMEM((4, (WIN + S) // 2, 128), U32),
        pltpu.VMEM((256, WIN + S), U32),
        pltpu.VMEM((1, S), F32),
        pltpu.VMEM((8, 384, 128), BF16),
        pltpu.VMEM((D, S), F32),
        pltpu.VMEM((96, D // 2, 128), U32),
        pltpu.VMEM((4, HB * DHB // 2, 128), U32),
        pltpu.VMEM((S, D), F32),
        pltpu.VMEM((MEM, D), F32),
        pltpu.VMEM((S + 16, 512), BF16),
        pltpu.VMEM((32, 16, 128), F32),
        pltpu.VMEM((D, S), BF16),
        pltpu.SemaphoreType.DMA((10,)),
    ]
    outT = pl.pallas_call(
        _kernel,
        out_shape=jax.ShapeDtypeStruct((D, S), BF16),
        in_specs=[any_spec] * 9,
        out_specs=any_spec,
        scratch_shapes=scratch,
        compiler_params=pltpu.CompilerParams(vmem_limit_bytes=110 * 1024 * 1024),
    )(xT, A_wqkv, A_wo, gate, mem0, B_Wq, B_Wk, B_Wv, woT)
    return outT.T[None]
```

```python
import functools
import jax
import jax.numpy as jnp
from jax import lax
import jax.experimental.pallas as pl
import jax.experimental.pallas.tpu as pltpu

F32 = jnp.float32
BF16 = jnp.bfloat16
U32 = jnp.uint32

S = 2048
D = 448
HA = 16
DHA = 28
DP = 32
WIN = 256
HB = 16
DHB = 256
MEM = 8
NBLK = S // 128
NPAIR = S // 64
NEG = -1e30
LOG2E = 1.4426950408889634

PV_AT = (-1, -1, -1)
OUT_AT = (16, 4)
SCORES_AT = ((5, 8, 11, 14), (8, 10, 12, 14), (5, 8, 11, 16))
FIN_AT = 7


def _dot(a, b):
    return jnp.dot(a, b, preferred_element_type=F32)


def _dot_nt(a, b):
    return lax.dot_general(a, b, (((1,), (1,)), ((), ())), preferred_element_type=F32)


def _pk(x):
    return pltpu.bitcast(x, U32)


def _upk(x):
    return pltpu.bitcast(x, BF16)


def _recip(x):
    r = pl.reciprocal(x, approx=True)
    return r * (2.0 - x * r)


def _cat(parts):
    return jnp.concatenate(parts, axis=0)


def _iota(shape, d):
    return lax.broadcasted_iota(jnp.int32, shape, d)


def _kernel(xT_hbm, wqkv_hbm, wo_hbm, gate_hbm, mem0_hbm, wq_hbm, wk_hbm, wv_hbm, woT_hbm,
            out_hbm,
            xT, wqkv_v, wo_v, gate_v, mem0_v, wraw, woT_raw,
            wT, woT_pad, QT, KA, VT, GT, PT, aT,
            W, WO, xb, mem_v, yb, OC, outT, sems):
    def cp(src, dst, i):
        return pltpu.make_async_copy(src, dst, sems.at[i])

    c_xs = [cp(xT_hbm.at[:, pl.ds(512 * i, 512)], xT.at[:, pl.ds(512 * i, 512)], 10 + i) for i in range(4)]
    c_wqkv = cp(wqkv_hbm, wqkv_v, 1)
    c_wo = cp(wo_hbm, wo_v, 2)
    c_gate = cp(gate_hbm, gate_v, 3)
    c_mem = cp(mem0_hbm, mem0_v, 4)
    c_wq = cp(wq_hbm, wraw.at[0], 5)
    c_wk = cp(wk_hbm, wraw.at[1], 6)
    c_wv = cp(wv_hbm, wraw.at[2], 7)
    c_woT = cp(woT_hbm, woT_raw, 8)
    for c in (c_wqkv, c_gate, c_xs[0], c_xs[1], c_wo, c_mem, c_xs[2], c_xs[3], c_woT, c_wq, c_wk, c_wv):
        c.start()

    c_wqkv.wait()
    c_gate.wait()
    wT[0:3 * D, :] = wqkv_v[...].T
    wT[3 * D:3 * D + 16, :] = _cat([gate_v[...].astype(F32), jnp.zeros((15, D), F32)]).astype(BF16)

    qscale = (DHA ** -0.5) * LOG2E
    for g in range(4):
        KA[g, 0:WIN // 2, :] = _pk(jnp.where(_iota((WIN, 128), 1) % DP == DHA, 1.0, 0.0).astype(BF16))
    VT[:, 0:WIN] = jnp.zeros((HA * DP // 2, WIN), U32)

    def a_scores(b, g, slot, units=(0, 1, 2, 3)):
        c0 = pl.multiple_of(b * 128, 128)
        upper = _iota((128, 128), 0) > _iota((128, 128), 1)
        for j in units:
            qj = QT[pl.ds(pl.multiple_of(g * 64 + j * 16, 16), 16), pl.ds(c0, 128)]
            parts = []
            if j > 0:
                parts.append(jnp.zeros((j * 16, 128), U32))
            parts.append(qj)
            if j < 3:
                parts.append(jnp.zeros(((3 - j) * 16, 128), U32))
            qm = _upk(_cat(parts))
            st = _cat([_dot(_upk(KA[g, pl.ds(pl.multiple_of(b * 64 + r * 48, 16), 48), :]), qm)
                       for r in range(4)])
            sm = jnp.where(upper, st[0:128], st[256:384])
            s1 = st[128:256]
            u = slot * 4 + j
            m = jnp.max(jnp.maximum(sm, s1), axis=0, keepdims=True)
            pm = jnp.exp2(sm - m)
            PT[u, 128:256, :] = jnp.exp2(s1 - m).astype(BF16)
            PT[u, 0:128, :] = jnp.where(upper, pm, 0.0).astype(BF16)
            PT[u, 256:384, :] = jnp.where(upper, 0.0, pm).astype(BF16)

    def a_pv(b, g, slot):
        c0 = pl.multiple_of(b * 128, 128)
        ots = []
        for j in range(4):
            vh = _upk(VT[pl.ds(pl.multiple_of(g * 64 + j * 16, 16), 16), pl.ds(c0, 384)])
            ot = _dot(vh, PT[slot * 4 + j])
            ot = ot * _recip(ot[DHA:DHA + 1, :])
            ots.append(ot.astype(BF16))
        return _cat(ots)

    def a_out(b, g, ot):
        c0 = pl.multiple_of(b * 128, 128)
        for r in range(4):
            w = _upk(woT_pad[g, r * 56:(r + 1) * 56, :])
            aT[r * 112:(r + 1) * 112, pl.ds(c0, 128)] += _dot(w, ot)

    def wprep16(i, blk):
        w = jnp.swapaxes(wraw[i, pl.ds(pl.multiple_of(blk * 16, 16), 16)], 0, 1)
        for h in range(HB):
            for t in range(2):
                W[i * 32 + h * 2 + t, pl.ds(pl.multiple_of(blk * 8, 8), 8), :] = _pk(w[h][:, t * 128:(t + 1) * 128])

    def woprep(h):
        woh = woT_raw[h].T
        r0 = pl.multiple_of(h * 128, 128)
        for n in range(3):
            WO[n, pl.ds(r0, 128), :] = _pk(woh[:, n * 128:(n + 1) * 128])
        WO[3, pl.ds(r0, 128), :] = _pk(jnp.concatenate(
            [woh[:, 384:448], jnp.zeros((256, 64), BF16)], axis=1))

    def proj_body(b, carry, extra=None, att0=None):
        if att0 is not None:
            u0 = (b - att0) * 2
            ot0 = a_pv(u0 // 4, u0 % 4, 0)
            ot1 = a_pv(u0 // 4, u0 % 4 + 1, 1)
            a_scores((u0 + 2) // 4, (u0 + 2) % 4, 0)
            a_scores((u0 + 2) // 4, (u0 + 2) % 4 + 1, 1)
        c0 = pl.multiple_of(b * 128, 128)
        xt = xT[:, pl.ds(c0, 128)]
        res = _dot(wT[...], xt)
        GT[:, pl.ds(c0, 128)] = res[3 * D:3 * D + 1, :]
        z3 = jnp.zeros((DP - DHA - 1, 128), F32)
        qpad = _cat([jnp.full((1, 128), NEG, F32), z3])
        kpad = jnp.zeros((DP - DHA, 128), F32)
        vpad = _cat([jnp.ones((1, 128), F32), z3])

        def padded(part, scale, pad):
            rows = []
            for h in range(HA):
                r = res[part * D + h * DHA:part * D + (h + 1) * DHA, :]
                rows.append(r if scale is None else r * scale)
                rows.append(pad)
            return _cat(rows)
        QT[:, pl.ds(c0, 128)] = _pk(padded(0, qscale, qpad).astype(BF16))
        k = padded(1, None, kpad).T.astype(BF16)
        for g in range(4):
            KA[g, pl.ds(pl.multiple_of(WIN // 2 + b * 64, 64), 64), :] = _pk(k[:, g * 128:(g + 1) * 128])
        VT[:, pl.ds(pl.multiple_of(WIN + c0, 128), 128)] = _pk(padded(2, None, vpad).astype(BF16))
        xb[pl.ds(c0, 128), :] = xt.astype(F32).T
        aT[:, pl.ds(c0, 128)] = jnp.zeros((D, 128), F32)
        yb[pl.ds(pl.multiple_of(16 + c0, 16), 128), :] = jnp.zeros((128, 512), BF16)
        if att0 is not None:
            a_out(u0 // 4, u0 % 4, ot0)
            a_out(u0 // 4, u0 % 4 + 1, ot1)
        if extra is not None:
            extra(b)
        return carry

    def ex_wo(b):
        for j in range(4):
            woprep((b - 4) * 4 + j)

    def mk_ex_w(i, b0):
        def ex(b):
            for j in range(7):
                wprep16(i, (b - b0) * 7 + j)
        return ex

    c_xs[0].wait()
    lax.fori_loop(0, 4, proj_body, 0)
    zpad = jnp.zeros((DP - DHA, D), F32)
    c_wo.wait()
    wo_f = wo_v[...].astype(F32)
    wo_rows = []
    for h in range(HA):
        wo_rows.append(wo_f[h * DHA:(h + 1) * DHA, :])
        wo_rows.append(zpad)
    woT_full = _cat(wo_rows).T.astype(BF16)
    for g in range(4):
        woT_pad[g] = _pk(woT_full[:, g * 128:(g + 1) * 128])
    c_xs[1].wait()
    c_woT.wait()
    lax.fori_loop(4, 8, functools.partial(proj_body, extra=ex_wo), 0)
    a_scores(0, 0, 0)
    a_scores(0, 1, 1)
    c_xs[2].wait()
    c_xs[3].wait()
    c_wq.wait()

    def att_body(b, carry):
        @pl.when(b == 12)
        def _():
            c_wk.wait()

        def ex(b):
            for j in range(7):
                wprep16((b - 8) // 4, (b % 4) * 7 + j)
        return proj_body(b, carry, extra=ex, att0=8)
    lax.fori_loop(8, 16, att_body, 0)

    c_mem.wait()
    mem_v[...] = mem0_v[...].astype(F32)
    c_wv.wait()
    a_scores(4, 2, 2)

    def wv_body(i, carry):
        for j in range(7):
            wprep16(2, i * 7 + j)
        return carry
    lax.fori_loop(0, 4, wv_body, 0)

    def qkv_pass(lhs, fill):
        res = []
        fill(-1)
        for h in range(HB):
            res.append([[_dot(lhs, _upk(W[i * 32 + h * 2 + t])) for t in range(2)] for i in range(3)])
            fill(h)
        return res

    def scores(q, k):
        return [_dot_nt(q[h][0], k[h][0]) + _dot_nt(q[h][1], k[h][1]) for h in range(HB)]

    def softmax(scs, valid):
        ps, rls = [], []
        for sc in scs:
            sc = jnp.where(valid, sc * (DHB ** -0.5 * LOG2E), NEG)
            m = jnp.max(sc, axis=1, keepdims=True)
            p = jnp.exp2(sc - m)
            ps.append(p.astype(BF16))
            rls.append(_recip(jnp.sum(p, axis=1, keepdims=True)))
        return ps, rls

    def pv(ps, rls, v):
        return [_dot(ps[h], v[h][t]) * rls[h] for h in range(HB) for t in range(2)]

    def o_pass(parts):
        acc = [None] * 4
        for c in range(8):
            lhs = jnp.concatenate(parts[4 * c:4 * c + 4], axis=1)
            for n in range(4):
                d = _dot(lhs, _upk(WO[n, c * 256:(c + 1) * 256, :]))
                acc[n] = d if acc[n] is None else acc[n] + d
        return jnp.concatenate(acc, axis=1)

    def fin(b):
        c0 = pl.multiple_of(b * 128, 128)
        bT = yb[pl.ds(pl.multiple_of(16 + c0, 16), 128), :].T[:D, :].astype(F32)
        g = jax.nn.sigmoid(GT[:, pl.ds(c0, 128)])
        outT[:, pl.ds(c0, 128)] = (g * aT[:, pl.ds(c0, 128)] + (1.0 - g) * bT).astype(BF16)

    def out_copy(b):
        c0 = pl.multiple_of(b * 128, 128)
        return pltpu.make_async_copy(outT.at[:, pl.ds(c0, 128)], out_hbm.at[:, pl.ds(c0, 128)], sems.at[9])

    def pair_body(p, carry_o, fills):
        i16, j48 = _iota((16, 48), 0), _iota((16, 48), 1)
        validA = (j48 < 40) & ((i16 < 8) | (j48 >= 32) | (j48 <= i16 - 8))
        i64, j80 = _iota((64, 80), 0), _iota((64, 80), 1)
        isA = (i64 >= 16) & (i64 < 40)
        posB = jnp.where(i64 < 8, 31, jnp.where(i64 < 16, i64 - 8, i64 - 32))
        validB = ((isA & (((j80 < 32) & (j80 <= i64 - 8)) | ((j80 >= 32) & (j80 < 40))))
                  | (jnp.logical_not(isA) & (((j80 >= 40) & (j80 < 72) & (j80 - 40 <= posB)) | (j80 >= 72))))
        r0 = pl.multiple_of(p * 64, 64)
        def per(fn):
            return [[fn(h, t) for t in range(2)] for h in range(HB)]

        fillA, fillB = fills
        lhsA = _cat([xb[pl.ds(r0, 32), :], mem_v[...], xb[pl.ds(r0 + 32, 8), :]]).astype(BF16)
        resA = qkv_pass(lhsA, fillA)
        kA = per(lambda h, t: resA[h][1][t].astype(BF16))
        vA = per(lambda h, t: resA[h][2][t].astype(BF16))
        qA = per(lambda h, t: _cat([resA[h][0][t][32:40], resA[h][0][t][0:8]]).astype(BF16))
        scA = scores(qA, kA)
        fillA(HB)
        oA = pv(*softmax(scA, validA), vA)
        outA = o_pass([_cat([oA[n], carry_o[n]]).astype(BF16) for n in range(32)])
        memA = outA[0:8, :D]
        yb[pl.ds(pl.multiple_of(16 + r0, 8), 8), :] = outA[8:16].astype(BF16)
        yb[pl.ds(r0, 16), :] = outA[16:32].astype(BF16)

        lhsB = _cat([xb[pl.ds(r0 + 40, 24), :], memA]).astype(BF16)
        resB = qkv_pass(lhsB, fillB)
        kB = per(lambda h, t: resB[h][1][t].astype(BF16))
        vB = per(lambda h, t: resB[h][2][t].astype(BF16))
        qB = per(lambda h, t: _cat([resB[h][0][t][24:32], resA[h][0][t][40:48],
                                    resA[h][0][t][8:32], resB[h][0][t][0:24]]).astype(BF16))
        kD = per(lambda h, t: _cat([kA[h][t], kB[h][t]]))
        vD = per(lambda h, t: _cat([vA[h][t], vB[h][t]]))
        scB = scores(qB, kD)
        oB = pv(*softmax(scB, validB), vD)
        outB = o_pass([o[0:48].astype(BF16) for o in oB])
        mem_v[...] = outB[0:8, :D]
        yb[pl.ds(pl.multiple_of(16 + r0 + 8, 8), 24), :] = outB[16:40].astype(BF16)
        yb[pl.ds(pl.multiple_of(16 + r0 + 32, 16), 16), :] = _cat([outB[8:16], outB[40:48]]).astype(BF16)
        return [o[48:64] for o in oB]

    NU = NBLK * 4

    def block_body(b, carry):
        bp = (b + NBLK - 1) % NBLK
        held = {}

        def mk_fill(j):
            u = 16 + 3 * b + j
            un = jnp.minimum(u + 3, NU - 1)

            def fill(h):
                if h == PV_AT[j]:
                    held[j] = a_pv(u // 4, u % 4, j)
                if j < 2 and h == OUT_AT[j]:
                    a_out(u // 4, u % 4, held[j])
                if h in SCORES_AT[j]:
                    a_scores(un // 4, un % 4, j, units=(SCORES_AT[j].index(h),))
                if j == 1 and h == FIN_AT:
                    fin(bp)
                    out_copy(bp).start()
            return fill

        def last_fill(h):
            if h == -1:
                u = 16 + 3 * b + 2
                a_out(u // 4, u % 4, held[2])

        co = [OC[n] for n in range(32)]
        co = pair_body(2 * b, co, (mk_fill(0), mk_fill(1)))
        co = pair_body(2 * b + 1, co, (mk_fill(2), last_fill))
        for n in range(32):
            OC[n] = co[n]
        return carry

    OC[...] = jnp.zeros((32, 16, 128), F32)
    lax.fori_loop(0, NBLK, block_body, 0)
    out_last = o_pass([OC[n].astype(BF16) for n in range(32)])
    yb[S:S + 16, :] = out_last.astype(BF16)
    for b in range(NBLK):
        out_copy(b).wait()
    fin(NBLK - 1)
    out_copy(NBLK - 1).start()
    out_copy(NBLK - 1).wait()


@jax.jit
def pallas_gated_mix__sliding_block__memory_aug_recurrent_mem_tr__prompt_kernel(
        A_x, A_wqkv, A_wo, B_x, B_mem0, B_Wq, B_Wk, B_Wv, B_Wo, B_seg_len, gate_w):
    xT = A_x[0].T
    mem0 = B_mem0[0]
    woT = B_Wo.transpose(0, 2, 1)
    gate = gate_w.reshape(1, D)
    any_spec = pl.BlockSpec(memory_space=pl.ANY)
    scratch = [
        pltpu.VMEM((D, S), BF16),
        pltpu.VMEM((D, 3 * D), BF16),
        pltpu.VMEM((D, D), BF16),
        pltpu.VMEM((1, D), BF16),
        pltpu.VMEM((MEM, D), BF16),
        pltpu.VMEM((3, D, HB, DHB), BF16),
        pltpu.VMEM((HB, D, DHB), BF16),
        pltpu.VMEM((3 * D + 16, D), BF16),
        pltpu.VMEM((4, D // 2, 128), U32),
        pltpu.VMEM((256, S), U32),
        pltpu.VMEM((4, (WIN + S) // 2, 128), U32),
        pltpu.VMEM((256, WIN + S), U32),
        pltpu.VMEM((1, S), F32),
        pltpu.VMEM((12, 384, 128), BF16),
        pltpu.VMEM((D, S), F32),
        pltpu.VMEM((96, D // 2, 128), U32),
        pltpu.VMEM((4, HB * DHB // 2, 128), U32),
        pltpu.VMEM((S, D), F32),
        pltpu.VMEM((MEM, D), F32),
        pltpu.VMEM((S + 16, 512), BF16),
        pltpu.VMEM((32, 16, 128), F32),
        pltpu.VMEM((D, S), BF16),
        pltpu.SemaphoreType.DMA((14,)),
    ]
    outT = pl.pallas_call(
        _kernel,
        out_shape=jax.ShapeDtypeStruct((D, S), BF16),
        in_specs=[any_spec] * 9,
        out_specs=any_spec,
        scratch_shapes=scratch,
        compiler_params=pltpu.CompilerParams(vmem_limit_bytes=110 * 1024 * 1024),
    )(xT, A_wqkv, A_wo, gate, mem0, B_Wq, B_Wk, B_Wv, woT)
    return outT.T[None]
```

```python
import jax
import jax.numpy as jnp
from jax import lax
import jax.experimental.pallas as pl
import jax.experimental.pallas.tpu as pltpu

F32 = jnp.float32
BF16 = jnp.bfloat16
U32 = jnp.uint32

S = 2048
D = 448
HA = 16
DHA = 28
DP = 32
WIN = 256
HB = 16
DHB = 256
MEM = 8
NBLK = S // 128
NEG = -1e30
LOG2E = 1.4426950408889634

PV_AT = (-1, -1, -1)
OUT_AT = (16, 4)
SCORES_AT = ((5, 8, 11, 14), (8, 10, 12, 14), (5, 8, 11, 16))
FIN_AT = 7


def _dot(a, b):
    return jnp.dot(a, b, preferred_element_type=F32)


def _dot_nt(a, b):
    return lax.dot_general(a, b, (((1,), (1,)), ((), ())), preferred_element_type=F32)


def _pk(x):
    return pltpu.bitcast(x, U32)


def _upk(x):
    return pltpu.bitcast(x, BF16)


def _recip(x):
    r = pl.reciprocal(x, approx=True)
    return r * (2.0 - x * r)


def _cat(parts):
    return jnp.concatenate(parts, axis=0)


def _iota(shape, d):
    return lax.broadcasted_iota(jnp.int32, shape, d)


def _kernel(xT_hbm, wqkv_hbm, wo_hbm, gate_hbm, mem0_hbm, wq_hbm, wk_hbm, wv_hbm, woT_hbm,
            out_hbm,
            xT, wqkv_v, wo_v, gate_v, mem0_v, wraw, woT_raw,
            wT, woT_pad, QT, KA, VT, GT, PT, aT,
            W, WO, xb, mem_v, yb, OC, outT, sems):
    def cp(src, dst, i):
        return pltpu.make_async_copy(src, dst, sems.at[i])

    c_xs = [cp(xT_hbm.at[:, pl.ds(512 * i, 512)], xT.at[:, pl.ds(512 * i, 512)], 10 + i) for i in range(4)]
    c_wqkv = cp(wqkv_hbm, wqkv_v, 1)
    c_wo = cp(wo_hbm, wo_v, 2)
    c_gate = cp(gate_hbm, gate_v, 3)
    c_mem = cp(mem0_hbm, mem0_v, 4)
    c_wq = cp(wq_hbm, wraw.at[0], 5)
    c_wk = cp(wk_hbm, wraw.at[1], 6)
    c_wv = cp(wv_hbm, wraw.at[2], 7)
    c_woT = cp(woT_hbm, woT_raw, 8)
    for c in (c_wqkv, c_gate, c_xs[0], c_xs[1], c_wo, c_mem, c_xs[2], c_xs[3], c_woT, c_wq, c_wk, c_wv):
        c.start()

    c_wqkv.wait()
    c_gate.wait()
    wT[0:3 * D, :] = wqkv_v[...].T
    wT[3 * D:3 * D + 16, :] = _cat([gate_v[...].astype(F32), jnp.zeros((15, D), F32)]).astype(BF16)

    qscale = (DHA ** -0.5) * LOG2E
    for g in range(4):
        KA[g, 0:WIN // 2, :] = _pk(jnp.where(_iota((WIN, 128), 1) % DP == DHA, 1.0, 0.0).astype(BF16))
    VT[:, 0:WIN] = jnp.zeros((HA * DP // 2, WIN), U32)

    def a_scores(b, g, slot, units=(0, 1, 2, 3)):
        c0 = pl.multiple_of(b * 128, 128)
        upper = _iota((128, 128), 0) > _iota((128, 128), 1)
        for j in units:
            qj = QT[pl.ds(pl.multiple_of(g * 64 + j * 16, 16), 16), pl.ds(c0, 128)]
            parts = []
            if j > 0:
                parts.append(jnp.zeros((j * 16, 128), U32))
            parts.append(qj)
            if j < 3:
                parts.append(jnp.zeros(((3 - j) * 16, 128), U32))
            qm = _upk(_cat(parts))
            st = _cat([_dot(_upk(KA[g, pl.ds(pl.multiple_of(b * 64 + r * 48, 16), 48), :]), qm)
                       for r in range(4)])
            sm = jnp.where(upper, st[0:128], st[256:384])
            s1 = st[128:256]
            u = slot * 4 + j
            m = jnp.max(jnp.maximum(sm, s1), axis=0, keepdims=True)
            pm = jnp.exp2(sm - m)
            PT[u, 128:256, :] = jnp.exp2(s1 - m).astype(BF16)
            PT[u, 0:128, :] = jnp.where(upper, pm, 0.0).astype(BF16)
            PT[u, 256:384, :] = jnp.where(upper, 0.0, pm).astype(BF16)

    def a_pv(b, g, slot):
        c0 = pl.multiple_of(b * 128, 128)
        ots = []
        for j in range(4):
            vh = _upk(VT[pl.ds(pl.multiple_of(g * 64 + j * 16, 16), 16), pl.ds(c0, 384)])
            ot = _dot(vh, PT[slot * 4 + j])
            ot = ot * _recip(ot[DHA:DHA + 1, :])
            ots.append(ot.astype(BF16))
        return _cat(ots)

    def a_out(b, g, ot):
        c0 = pl.multiple_of(b * 128, 128)
        for r in range(4):
            w = _upk(woT_pad[g, r * 56:(r + 1) * 56, :])
            aT[r * 112:(r + 1) * 112, pl.ds(c0, 128)] += _dot(w, ot)

    def wprep16(i, blk):
        w = jnp.swapaxes(wraw[i, pl.ds(pl.multiple_of(blk * 16, 16), 16)], 0, 1)
        for h in range(HB):
            for t in range(2):
                W[i * 32 + h * 2 + t, pl.ds(pl.multiple_of(blk * 8, 8), 8), :] = _pk(w[h][:, t * 128:(t + 1) * 128])

    def woprep(h):
        woh = woT_raw[h].T
        r0 = pl.multiple_of(h * 128, 128)
        for n in range(3):
            WO[n, pl.ds(r0, 128), :] = _pk(woh[:, n * 128:(n + 1) * 128])
        WO[3, pl.ds(r0, 128), :] = _pk(jnp.concatenate(
            [woh[:, 384:448], jnp.zeros((256, 64), BF16)], axis=1))

    def proj_body(b, carry, extra=None, att0=None):
        if att0 is not None:
            u0 = (b - att0) * 2
            ot0 = a_pv(u0 // 4, u0 % 4, 0)
            ot1 = a_pv(u0 // 4, u0 % 4 + 1, 1)
            a_scores((u0 + 2) // 4, (u0 + 2) % 4, 0)
            a_scores((u0 + 2) // 4, (u0 + 2) % 4 + 1, 1)
        c0 = pl.multiple_of(b * 128, 128)
        xt = xT[:, pl.ds(c0, 128)]
        res = _dot(wT[...], xt)
        GT[:, pl.ds(c0, 128)] = res[3 * D:3 * D + 1, :]
        z3 = jnp.zeros((DP - DHA - 1, 128), F32)
        qpad = _cat([jnp.full((1, 128), NEG, F32), z3])
        kpad = jnp.zeros((DP - DHA, 128), F32)
        vpad = _cat([jnp.ones((1, 128), F32), z3])

        def padded(part, scale, pad):
            rows = []
            for h in range(HA):
                r = res[part * D + h * DHA:part * D + (h + 1) * DHA, :]
                rows.append(r if scale is None else r * scale)
                rows.append(pad)
            return _cat(rows)
        QT[:, pl.ds(c0, 128)] = _pk(padded(0, qscale, qpad).astype(BF16))
        k = padded(1, None, kpad).T.astype(BF16)
        for g in range(4):
            KA[g, pl.ds(pl.multiple_of(WIN // 2 + b * 64, 64), 64), :] = _pk(k[:, g * 128:(g + 1) * 128])
        VT[:, pl.ds(pl.multiple_of(WIN + c0, 128), 128)] = _pk(padded(2, None, vpad).astype(BF16))
        xb[pl.ds(c0, 128), :] = xt.astype(F32).T
        aT[:, pl.ds(c0, 128)] = jnp.zeros((D, 128), F32)
        yb[pl.ds(pl.multiple_of(16 + c0, 16), 128), :] = jnp.zeros((128, 512), BF16)
        if att0 is not None:
            a_out(u0 // 4, u0 % 4, ot0)
            a_out(u0 // 4, u0 % 4 + 1, ot1)
        if extra is not None:
            extra(b)
        return carry

    def plain_body(b, carry):
        @pl.when(b == 4)
        def _():
            c_xs[1].wait()
        return proj_body(b, carry)

    c_xs[0].wait()
    lax.fori_loop(0, 8, plain_body, 0)
    zpad = jnp.zeros((DP - DHA, D), F32)
    c_wo.wait()
    wo_f = wo_v[...].astype(F32)
    wo_rows = []
    for h in range(HA):
        wo_rows.append(wo_f[h * DHA:(h + 1) * DHA, :])
        wo_rows.append(zpad)
    woT_full = _cat(wo_rows).T.astype(BF16)
    for g in range(4):
        woT_pad[g] = _pk(woT_full[:, g * 128:(g + 1) * 128])
    a_scores(0, 0, 0)
    a_scores(0, 1, 1)
    c_xs[2].wait()
    c_xs[3].wait()
    c_woT.wait()
    c_wq.wait()

    def att_body(b, carry):
        @pl.when(b == 12)
        def _():
            c_wk.wait()

        def ex(b):
            for j in range(2):
                woprep((b - 8) * 2 + j)
            for j in range(7):
                wprep16((b - 8) // 4, (b % 4) * 7 + j)
        return proj_body(b, carry, extra=ex, att0=8)
    lax.fori_loop(8, 16, att_body, 0)

    c_mem.wait()
    mem_v[...] = mem0_v[...].astype(F32)
    c_wv.wait()
    a_scores(4, 2, 2)

    def wv_body(i, carry):
        for j in range(7):
            wprep16(2, i * 7 + j)
        return carry
    lax.fori_loop(0, 4, wv_body, 0)

    def qkv_pass(lhs, fill):
        res = []
        fill(-1)
        for h in range(HB):
            res.append([[_dot(lhs, _upk(W[i * 32 + h * 2 + t])) for t in range(2)] for i in range(3)])
            fill(h)
        return res

    def scores(q, k):
        return [_dot_nt(q[h][0], k[h][0]) + _dot_nt(q[h][1], k[h][1]) for h in range(HB)]

    def softmax(scs, valid):
        ps, rls = [], []
        for sc in scs:
            sc = jnp.where(valid, sc * (DHB ** -0.5 * LOG2E), NEG)
            m = jnp.max(sc, axis=1, keepdims=True)
            p = jnp.exp2(sc - m)
            ps.append(p.astype(BF16))
            rls.append(_recip(jnp.sum(p, axis=1, keepdims=True)))
        return ps, rls

    def pv(ps, rls, v):
        return [_dot(ps[h], v[h][t]) * rls[h] for h in range(HB) for t in range(2)]

    def o_pass(parts):
        acc = [None] * 4
        for c in range(8):
            lhs = jnp.concatenate(parts[4 * c:4 * c + 4], axis=1)
            for n in range(4):
                d = _dot(lhs, _upk(WO[n, c * 256:(c + 1) * 256, :]))
                acc[n] = d if acc[n] is None else acc[n] + d
        return jnp.concatenate(acc, axis=1)

    def fin(b):
        c0 = pl.multiple_of(b * 128, 128)
        bT = yb[pl.ds(pl.multiple_of(16 + c0, 16), 128), :].T[:D, :].astype(F32)
        g = jax.nn.sigmoid(GT[:, pl.ds(c0, 128)])
        outT[:, pl.ds(c0, 128)] = (g * aT[:, pl.ds(c0, 128)] + (1.0 - g) * bT).astype(BF16)

    def out_copy(b):
        c0 = pl.multiple_of(b * 128, 128)
        return pltpu.make_async_copy(outT.at[:, pl.ds(c0, 128)], out_hbm.at[:, pl.ds(c0, 128)], sems.at[9])

    def pair_body(p, carry_o, fills):
        i16, j48 = _iota((16, 48), 0), _iota((16, 48), 1)
        validA = (j48 < 40) & ((i16 < 8) | (j48 >= 32) | (j48 <= i16 - 8))
        i64, j80 = _iota((64, 80), 0), _iota((64, 80), 1)
        isA = (i64 >= 16) & (i64 < 40)
        posB = jnp.where(i64 < 8, 31, jnp.where(i64 < 16, i64 - 8, i64 - 32))
        validB = ((isA & (((j80 < 32) & (j80 <= i64 - 8)) | ((j80 >= 32) & (j80 < 40))))
                  | (jnp.logical_not(isA) & (((j80 >= 40) & (j80 < 72) & (j80 - 40 <= posB)) | (j80 >= 72))))
        r0 = pl.multiple_of(p * 64, 64)
        def per(fn):
            return [[fn(h, t) for t in range(2)] for h in range(HB)]

        fillA, fillB = fills
        lhsA = _cat([xb[pl.ds(r0, 32), :], mem_v[...], xb[pl.ds(r0 + 32, 8), :]]).astype(BF16)
        resA = qkv_pass(lhsA, fillA)
        kA = per(lambda h, t: resA[h][1][t].astype(BF16))
        vA = per(lambda h, t: resA[h][2][t].astype(BF16))
        qA = per(lambda h, t: _cat([resA[h][0][t][32:40], resA[h][0][t][0:8]]).astype(BF16))
        scA = scores(qA, kA)
        fillA(HB)
        oA = pv(*softmax(scA, validA), vA)
        outA = o_pass([_cat([oA[n], carry_o[n]]).astype(BF16) for n in range(32)])
        memA = outA[0:8, :D]
        yb[pl.ds(pl.multiple_of(16 + r0, 8), 8), :] = outA[8:16].astype(BF16)
        yb[pl.ds(r0, 16), :] = outA[16:32].astype(BF16)

        lhsB = _cat([xb[pl.ds(r0 + 40, 24), :], memA]).astype(BF16)
        resB = qkv_pass(lhsB, fillB)
        kB = per(lambda h, t: resB[h][1][t].astype(BF16))
        vB = per(lambda h, t: resB[h][2][t].astype(BF16))
        qB = per(lambda h, t: _cat([resB[h][0][t][24:32], resA[h][0][t][40:48],
                                    resA[h][0][t][8:32], resB[h][0][t][0:24]]).astype(BF16))
        kD = per(lambda h, t: _cat([kA[h][t], kB[h][t]]))
        vD = per(lambda h, t: _cat([vA[h][t], vB[h][t]]))
        scB = scores(qB, kD)
        oB = pv(*softmax(scB, validB), vD)
        outB = o_pass([o[0:48].astype(BF16) for o in oB])
        mem_v[...] = outB[0:8, :D]
        yb[pl.ds(pl.multiple_of(16 + r0 + 8, 8), 24), :] = outB[16:40].astype(BF16)
        yb[pl.ds(pl.multiple_of(16 + r0 + 32, 16), 16), :] = _cat([outB[8:16], outB[40:48]]).astype(BF16)
        return [o[48:64] for o in oB]

    NU = NBLK * 4

    def block_body(b, carry):
        bp = (b + NBLK - 1) % NBLK
        held = {}

        def mk_fill(j):
            u = 16 + 3 * b + j
            un = jnp.minimum(u + 3, NU - 1)

            def fill(h):
                if h == PV_AT[j]:
                    held[j] = a_pv(u // 4, u % 4, j)
                if j < 2 and h == OUT_AT[j]:
                    a_out(u // 4, u % 4, held[j])
                if h in SCORES_AT[j]:
                    a_scores(un // 4, un % 4, j, units=(SCORES_AT[j].index(h),))
                if j == 1 and h == FIN_AT:
                    fin(bp)
                    out_copy(bp).start()
            return fill

        def last_fill(h):
            if h == -1:
                u = 16 + 3 * b + 2
                a_out(u // 4, u % 4, held[2])

        co = [OC[n] for n in range(32)]
        co = pair_body(2 * b, co, (mk_fill(0), mk_fill(1)))
        co = pair_body(2 * b + 1, co, (mk_fill(2), last_fill))
        for n in range(32):
            OC[n] = co[n]
        return carry

    OC[...] = jnp.zeros((32, 16, 128), F32)
    lax.fori_loop(0, NBLK, block_body, 0)
    out_last = o_pass([OC[n].astype(BF16) for n in range(32)])
    yb[S:S + 16, :] = out_last.astype(BF16)
    for b in range(NBLK):
        out_copy(b).wait()
    fin(NBLK - 1)
    out_copy(NBLK - 1).start()
    out_copy(NBLK - 1).wait()


@jax.jit
def pallas_gated_mix__sliding_block__memory_aug_recurrent_mem_tr__prompt_kernel(
        A_x, A_wqkv, A_wo, B_x, B_mem0, B_Wq, B_Wk, B_Wv, B_Wo, B_seg_len, gate_w):
    xT = A_x[0].T
    mem0 = B_mem0[0]
    woT = B_Wo.transpose(0, 2, 1)
    gate = gate_w.reshape(1, D)
    any_spec = pl.BlockSpec(memory_space=pl.ANY)
    scratch = [
        pltpu.VMEM((D, S), BF16),
        pltpu.VMEM((D, 3 * D), BF16),
        pltpu.VMEM((D, D), BF16),
        pltpu.VMEM((1, D), BF16),
        pltpu.VMEM((MEM, D), BF16),
        pltpu.VMEM((3, D, HB, DHB), BF16),
        pltpu.VMEM((HB, D, DHB), BF16),
        pltpu.VMEM((3 * D + 16, D), BF16),
        pltpu.VMEM((4, D // 2, 128), U32),
        pltpu.VMEM((256, S), U32),
        pltpu.VMEM((4, (WIN + S) // 2, 128), U32),
        pltpu.VMEM((256, WIN + S), U32),
        pltpu.VMEM((1, S), F32),
        pltpu.VMEM((12, 384, 128), BF16),
        pltpu.VMEM((D, S), F32),
        pltpu.VMEM((96, D // 2, 128), U32),
        pltpu.VMEM((4, HB * DHB // 2, 128), U32),
        pltpu.VMEM((S, D), F32),
        pltpu.VMEM((MEM, D), F32),
        pltpu.VMEM((S + 16, 512), BF16),
        pltpu.VMEM((32, 16, 128), F32),
        pltpu.VMEM((D, S), BF16),
        pltpu.SemaphoreType.DMA((14,)),
    ]
    outT = pl.pallas_call(
        _kernel,
        out_shape=jax.ShapeDtypeStruct((D, S), BF16),
        in_specs=[any_spec] * 9,
        out_specs=any_spec,
        scratch_shapes=scratch,
        compiler_params=pltpu.CompilerParams(vmem_limit_bytes=110 * 1024 * 1024),
    )(xT, A_wqkv, A_wo, gate, mem0, B_Wq, B_Wk, B_Wv, woT)
    return outT.T[None]
```
